```python
import jax
import jax.numpy as jnp

def _softmax(x, axis=-1):
    return jax.nn.softmax(x, axis=axis)
def _gelu(x):
    return jax.nn.gelu(x, approximate=True)
def _silu(x):
    return jax.nn.silu(x)
def _sigmoid(x):
    return jax.nn.sigmoid(x)
def _layernorm(x, axis=-1, eps=1e-5):
    m = jnp.mean(x, axis=axis, keepdims=True)
    v = jnp.var(x, axis=axis, keepdims=True)
    return (x - m) / jnp.sqrt(v + eps)
def _scatter_add(tgt, idx, src, axis=0):
    return tgt.at[idx].add(src)
def _segment_sum(src, seg, n):
    return jax.ops.segment_sum(src, seg, n)
class _Rng:
    def __init__(self, key):
        self._k = key
    def _next(self):
        self._k, sub = jax.random.split(self._k)
        return sub
    def normal(self, shape):
        return jax.random.normal(self._next(), shape, dtype=jnp.bfloat16)
    def randint(self, lo, hi, shape):
        return jax.random.randint(self._next(), shape, lo, hi, dtype=jnp.int32)
    def uniform(self, shape, lo=0.0, hi=1.0):
        return jax.random.uniform(self._next(), shape, jnp.bfloat16, lo, hi)
    def permutation(self, n):
        return jax.random.permutation(self._next(), n)


kernel_name = 'standalone__gqa_block_cached__near_ridge'

def _fwd_setup_inputs():
    _rng = _Rng(jax.random.key(int.from_bytes(__import__("os").urandom(4), "little")))
    _w = (lambda a: (lambda t: t.astype(jnp.bfloat16) if jnp.issubdtype(t.dtype, jnp.floating) else t)(jnp.asarray(a)))
    B, Sq, D = 16, 64, 640
    Hq, Hkv, Sk, Dh = 32, 32, 512, 192
    assert Hq % Hkv == 0, (Hq, Hkv)
    return {
        "x": _w((lambda *s: _rng.normal(s) * 0.05)(B, Sq, D)),
        "k_cache": _w((lambda *s: _rng.normal(s) * 0.05)(B, Hkv, Sk, Dh)),
        "v_cache": _w((lambda *s: _rng.normal(s) * 0.05)(B, Hkv, Sk, Dh)),
        "wq": _w((lambda *s: _rng.normal(s) * 0.05)(D, Hq * Dh) * (D ** -0.5)),
        "wo": _w((lambda *s: _rng.normal(s) * 0.05)(Hq * Dh, D) * ((Hq * Dh) ** -0.5)),
    }

def _fwd_reference(x, k_cache, v_cache, wq, wo):
    B, Sq, D = x.shape
    Hq, Dh = 32, 192
    Hkv = k_cache.shape[1]
    rep = Hq // Hkv
    q = (lambda x, *d: x.transpose(*d))((x @ wq).reshape(B, Sq, Hq, Dh), 0, 2, 1, 3)
    k = jnp.repeat(k_cache, rep, axis=1)
    v = jnp.repeat(v_cache, rep, axis=1)
    scores = jnp.einsum("bhqd,bhkd->bhqk", q, k) * (Dh ** -0.5)
    p = _softmax(scores, axis=-1)
    o = jnp.einsum("bhqk,bhkd->bhqd", p, v)
    return (lambda x, *d: x.transpose(*d))(o, 0, 2, 1, 3).reshape(B, Sq, Hq * Dh) @ wo


def setup_inputs():
    _inp = _fwd_setup_inputs()
    _gk = jax.random.fold_in(jax.random.key(int.from_bytes(__import__("os").urandom(4), "little")), 2**31 - 1)
    _shapes = [[16, 64, 640]]
    _dtypes = ['bfloat16']
    _gks = jax.random.split(_gk, len(_shapes))
    _gs = [jax.random.normal(k, s, dtype=jnp.dtype(d)) * 0.05 for k, s, d in zip(_gks, _shapes, _dtypes)]
    _inp["grad_out"] = _gs[0]
    return _inp

def reference(x, k_cache, v_cache, wq, wo, grad_out):
    _const = dict()
    def _f(*_d):
        return _fwd_reference(**{'x': _d[0], 'k_cache': _d[1], 'v_cache': _d[2], 'wq': _d[3], 'wo': _d[4], **_const})
    _out, _vjp = jax.vjp(_f, x, k_cache, v_cache, wq, wo)
    _grads = _vjp(grad_out)
    _out0 = jnp.asarray(_out)
    return (_out0, *[jnp.asarray(_g) for _g in _grads])
```

```python
import functools
import math

import jax
import jax.numpy as jnp
from jax import lax
import jax.experimental.pallas as pl
import jax.experimental.pallas.tpu as pltpu

F32 = jnp.float32
BF16 = jnp.bfloat16
_NT = (((1,), (1,)), ((), ()))
_TN = (((0,), (0,)), ((), ()))

B, SQ, D = 16, 64, 640
H, SK, DH = 32, 512, 192
HP = 2 * DH
NS = H // 2


def _dot(a, b):
    return jnp.dot(a, b, preferred_element_type=F32)


def _dot_nt(a, b):
    return lax.dot_general(a, b, _NT, preferred_element_type=F32)


def _dot_tn(a, b):
    return lax.dot_general(a, b, _TN, preferred_element_type=F32)


def make(G=2, pro=2, wsched=(0, 0, 1, 2), wnb=4, wrows=32, rd_it=None, compute=True, dma=True, early=True, flags=None):
    NI = B // G
    T = G * SQ
    rd_it = NI // 2 if rd_it is None else rd_it
    scale = DH ** -0.5

    def body(slot, it, first_s, x_v, g_v, k_v, v_v, wq_v, wo_v, dk_v, dv_v, dwq_s, dwo_s,
             out_s, dx_s, out_a, dx_a, dwq_a, dwo_a):
        tok = pl.ds(pl.multiple_of(it * T, T), T)
        lo = lax.broadcasted_iota(jnp.int32, (SQ, 128), 1) < 64
        xb = x_v[tok, :]
        gb = g_v[tok, :]
        q = _dot(xb, wq_v[slot]) * scale
        do = _dot_nt(gb, wo_v[slot])

        def split(a, j):
            a = a[j * SQ:(j + 1) * SQ]
            m = a[:, 128:256]
            mid = jnp.concatenate([jnp.where(lo, m, 0.0), jnp.where(lo, 0.0, m)], 0)
            return a[:, 0:128].astype(BF16), mid.astype(BF16), a[:, 256:384].astype(BF16)

        def scores(parts, w):
            a0, am, a2 = parts
            mid = _dot(am, w[128:256, :])
            return jnp.concatenate([_dot(a0, w[0:128, :]) + mid[0:SQ],
                                    _dot(a2, w[256:384, :]) + mid[SQ:]], 0)

        def apply(pb, w):
            mid = _dot_nt(pb, w[128:256, :])
            return jnp.concatenate([_dot_nt(pb[0:SQ], w[0:128, :]),
                                    jnp.where(lo, mid[0:SQ], mid[SQ:]),
                                    _dot_nt(pb[SQ:], w[256:384, :])], 1)

        def blockdiag(parts):
            a0, am, a2 = parts
            z = jnp.zeros_like(a0)
            return jnp.concatenate([jnp.concatenate([a0, z], 0), am, jnp.concatenate([z, a2], 0)], 1)

        kr = [k_v.at[slot, it * G + j] for j in range(G)]
        vr = [v_v.at[slot, it * G + j] for j in range(G)]
        qp = [split(q, j) for j in range(G)]
        dop = [split(do, j) for j in range(G)]
        s = [scores(qp[j], kr[j]) for j in range(G)]
        dp = [scores(dop[j], vr[j]) for j in range(G)]
        p = []
        for j in range(G):
            e = jnp.exp(s[j] - jnp.max(s[j], axis=1, keepdims=True))
            p.append(e * (1.0 / jnp.sum(e, axis=1, keepdims=True)))
        o = []
        for j in range(G):
            pb = p[j].astype(BF16)
            o.append(apply(pb, vr[j]))
            dv_v[slot, it * G + j] = _dot_tn(blockdiag(dop[j]), pb).astype(BF16)
        dsb = []
        for j in range(G):
            delta = jnp.sum(p[j] * dp[j], axis=1, keepdims=True)
            dsb.append((p[j] * (dp[j] - delta)).astype(BF16))
        dq = [apply(dsb[j], kr[j]) * scale for j in range(G)]
        for j in range(G):
            dk_v[slot, it * G + j] = _dot_tn(blockdiag(qp[j]), dsb[j]).astype(BF16)
        ob = jnp.concatenate(o, 0).astype(BF16)
        dqb = jnp.concatenate(dq, 0).astype(BF16)

        def accumulate(acc, idx, stage, sidx, fresh, val):
            new = jnp.where(fresh, 0.0, acc[idx]) + val
            acc[idx] = new
            stage[sidx] = new.astype(BF16)

        accumulate(out_a, (tok,), out_s, (tok,), first_s, _dot(ob, wo_v[slot]))
        accumulate(dwo_a, ..., dwo_s, slot, it == 0, _dot_tn(ob, gb))
        accumulate(dx_a, (tok,), dx_s, (tok,), first_s, _dot_nt(dqb, wq_v[slot]))
        accumulate(dwq_a, ..., dwq_s, slot, it == 0, _dot_tn(xb, dqb))

    def kernel(x_h, k_h, v_h, wq_h, wo_h, g_h, out_h, dx_h, dk_h, dv_h, dwq_h, dwo_h,
               x_v, g_v, k_v, v_v, wq_v, wo_v, dk_v, dv_v, dwq_s, dwo_s, out_s, dx_s,
               out_a, dx_a, dwq_a, dwo_a, rsem, rwsem, wsem, wlsem, xsem, fsem):
        def hrows(s):
            return pl.ds(pl.multiple_of(s * HP, HP), HP)

        def rd_w(s):
            sl = s % 2
            return [pltpu.make_async_copy(wq_h.at[:, hrows(s)], wq_v.at[sl], rwsem.at[sl]),
                    pltpu.make_async_copy(wo_h.at[hrows(s), :], wo_v.at[sl], rwsem.at[sl])]

        def rd_kv(s, i):
            sl = s % 2
            bs = pl.ds(i * G, G)
            return [pltpu.make_async_copy(src.at[bs, hrows(s)], dst.at[sl, bs], rsem.at[sl * NI + i])
                    for src, dst in ((k_h, k_v), (v_h, v_v))]

        def rd_x(i):
            tok = pl.ds(pl.multiple_of(i * T, T), T)
            return [pltpu.make_async_copy(src.at[tok], dst.at[tok], xsem.at[i])
                    for src, dst in ((x_h, x_v), (g_h, g_v))]

        def wr_kv(s, b0, nb, rows, sem):
            sl = s % 2
            bs = pl.ds(b0, nb)
            return [pltpu.make_async_copy(
                src.at[sl, bs, pl.ds(c * rows, rows)],
                dst.at[bs, pl.ds(pl.multiple_of(s * HP + c * rows, rows), rows)], sem)
                for c in range(HP // rows) for src, dst in ((dk_v, dk_h), (dv_v, dv_h))]

        def wr_w(s, sem_q, sem_o):
            sl = s % 2
            return [pltpu.make_async_copy(dwq_s.at[sl], dwq_h.at[:, hrows(s)], sem_q),
                    pltpu.make_async_copy(dwo_s.at[sl], dwo_h.at[hrows(s), :], sem_o)]

        def wr_x(i, sem):
            tok = pl.ds(pl.multiple_of(i * T, T), T)
            return [pltpu.make_async_copy(src.at[tok], dst.at[tok], sem)
                    for src, dst in ((out_s, out_h), (dx_s, dx_h))]

        if dma in ("init", "zero"):
            if dma == "init":
                cs = rd_w(0) + rd_w(1)
                for i in range(NI):
                    cs += rd_x(i) + rd_kv(0, i) + rd_kv(1, i)
                for c in cs:
                    c.start()
                for c in cs:
                    c.wait()
            else:
                for r in (x_v, g_v, wq_v, wo_v):
                    r[...] = jnp.zeros(r.shape, r.dtype)
                def z(i, _):
                    for r in (k_v, v_v):
                        r[i // B, i % B] = jnp.zeros(r.shape[2:], r.dtype)
                lax.fori_loop(0, 2 * B, z, None)

        def keep(c):
            if dma in ("init", "zero"):
                return False
            if dma in (True, False):
                return dma
            is_w = any(c.dst_sem is m for m in (wsem, wlsem, fsem))
            return is_w == (dma == "w")

        def start(cs):
            for c in cs:
                if keep(c):
                    c.start()

        def wait(cs):
            for c in cs:
                if keep(c):
                    c.wait()

        def whole(ref, sem):
            return [pltpu.make_async_copy(ref, ref, sem)]

        start(rd_x(0)[:1] + rd_w(0) + rd_x(0)[1:] + rd_kv(0, 0))
        def rest0():
            for i in range(1, NI):
                start(rd_x(i) + rd_kv(0, i))

        def rest1():
            start(rd_w(1))
            for i in range(NI):
                start(rd_kv(1, i))

        if pro < 2:
            rest0()
        if pro < 1:
            rest1()

        def step(n, _):
            s = n // NI
            it = n % NI
            sl = s % 2

            def issue_writes(at):
                for gi, a in enumerate(wsched):
                    if a == at:
                        start(wr_kv(s - 1, gi * wnb, wnb, wrows, wsem))
                if at == max(wsched):
                    start(wr_w(s - 1, wsem, wlsem))

            @pl.when(s == 0)
            def _():
                @pl.when(it == 0)
                def _():
                    wait(rd_w(0))
                    if pro >= 2:
                        rest0()
                if pro >= 1:
                    pl.when(it == 1)(rest1)
                wait(rd_x(it) + rd_kv(0, it))

            @pl.when(jnp.logical_and(s > 0, it == 0))
            def _():
                wait(rd_w(s))
                last = rd_kv(s, NI - 1)
                for i in range(NI - 1):
                    wait(rd_kv(s, i))
                wait(last[:1] if early else last)
                issue_writes(0)
                if early:
                    wait(last[1:])

            for at in sorted(set(wsched) - {0}):
                pl.when(jnp.logical_and(s > 0, it == at))(functools.partial(issue_writes, at))

            @pl.when(jnp.logical_and(jnp.logical_and(s > 0, s < NS - 1), it == rd_it))
            def _():
                ww = wr_w(s - 1, wsem, wlsem)
                wait(whole(dk_v.at[1 - sl], wsem) + whole(dv_v.at[1 - sl], wsem) + ww[:1])
                if not early:
                    wait(ww[1:])
                start(rd_w(s + 1))
                for i in range(NI):
                    start(rd_kv(s + 1, i))
                if early:
                    wait(ww[1:])

            if compute:
                body(sl, it, s == 0, x_v, g_v, k_v, v_v, wq_v, wo_v, dk_v, dv_v, dwq_s, dwo_s,
                     out_s, dx_s, out_a, dx_a, dwq_a, dwo_a)

            @pl.when(s == NS - 1)
            def _():
                start(wr_kv(NS - 1, it * G, G, wrows, fsem) + wr_x(it, fsem))

        lax.fori_loop(0, NS * NI, step, None)
        start(wr_w(NS - 1, fsem, fsem))
        sl = (NS - 2) % 2
        wait(whole(dk_v.at[sl], wsem) + whole(dv_v.at[sl], wsem) + wr_w(NS - 2, wsem, wlsem))
        sl = (NS - 1) % 2
        wait(whole(dk_v.at[sl], fsem) + whole(dv_v.at[sl], fsem) + whole(out_s, fsem) + whole(dx_s, fsem)
             + wr_w(NS - 1, fsem, fsem))

    @jax.jit
    def run(x, k_cache, v_cache, wq, wo, grad_out):
        kt = jnp.swapaxes(k_cache, 2, 3).reshape(B, H * DH, SK)
        vt = jnp.swapaxes(v_cache, 2, 3).reshape(B, H * DH, SK)
        hbm = pl.BlockSpec(memory_space=pl.ANY)
        tok = jax.ShapeDtypeStruct((B * SQ, D), BF16)
        kv = jax.ShapeDtypeStruct((B, H * DH, SK), BF16)
        out, dx, dkt, dvt, dwq, dwo = pl.pallas_call(
            kernel,
            in_specs=[hbm] * 6,
            out_specs=[hbm] * 6,
            out_shape=[tok, tok, kv, kv, jax.ShapeDtypeStruct(wq.shape, BF16),
                       jax.ShapeDtypeStruct(wo.shape, BF16)],
            scratch_shapes=[
                pltpu.VMEM((B * SQ, D), BF16), pltpu.VMEM((B * SQ, D), BF16),
                pltpu.VMEM((2, B, HP, SK), BF16), pltpu.VMEM((2, B, HP, SK), BF16),
                pltpu.VMEM((2, D, HP), BF16), pltpu.VMEM((2, HP, D), BF16),
                pltpu.VMEM((2, B, HP, SK), BF16), pltpu.VMEM((2, B, HP, SK), BF16),
                pltpu.VMEM((2, D, HP), BF16), pltpu.VMEM((2, HP, D), BF16),
                pltpu.VMEM((B * SQ, D), BF16), pltpu.VMEM((B * SQ, D), BF16),
                pltpu.VMEM((B * SQ, D), F32), pltpu.VMEM((B * SQ, D), F32),
                pltpu.VMEM((D, HP), F32), pltpu.VMEM((HP, D), F32),
                pltpu.SemaphoreType.DMA((2 * NI,)), pltpu.SemaphoreType.DMA((2,)),
                pltpu.SemaphoreType.DMA, pltpu.SemaphoreType.DMA,
                pltpu.SemaphoreType.DMA((NI,)), pltpu.SemaphoreType.DMA,
            ],
            compiler_params=pltpu.CompilerParams(vmem_limit_bytes=110 * 2 ** 20, flags=flags, disable_bounds_checks=True),
        )(x.reshape(B * SQ, D), kt, vt, wq, wo, grad_out.reshape(B * SQ, D))
        unt = lambda a: jnp.swapaxes(a.reshape(B, H, DH, SK), 2, 3)
        return out.reshape(B, SQ, D), dx.reshape(B, SQ, D), unt(dkt), unt(dvt), dwq, dwo

    return run


pallas_standalone__gqa_block_cached__near_ridge_kernel = make()
```

```python
import jax
import jax.numpy as jnp
from jax import lax
import jax.experimental.pallas as pl
import jax.experimental.pallas.tpu as pltpu

F32 = jnp.float32
BF16 = jnp.bfloat16

B, SQ, D = 16, 64, 640
H, SK, DH = 32, 512, 192
HP = 2 * DH
NS = H // 2
G = 8
T = G * SQ
N = NS * B // G
GB = 4
NG = NS * B // GB
RQ, WQ = 4, 2
NR, NW = 14, 16
NWS = 8
FIRST = 4
SKEW = 27
WRITE_CUTS = (0, 24, 88, 152, 216, 280, 344, 384)
TAIL_WIDTHS = ((256, 256, 256, 256), (256, 256, 128, 128, 128))

ORDER = """
q01 do01 S0 q23 do23 W R OV0 dP0 S1 q45 E W R QK0 OV1 dP1 do45 R S2 QK1 W OV2 dP2 out01 R S3 R W QK2 OV3 R dP3 dx01
W S4 QK3 R OV4 R dP4 S5 q67 E QK4 W R OV5 dP5 do67 S6 R R QK5 OV6 W dP6 S7 out23 R OV7 dP7 QK6 dx23 R W QK7 W out45
R dx45 out67 R pin dx67 W fin dwq R dwo R
"""
FIRST_ORDER = """
in0 P q01 q23 q45 q67 in1 P do01 do23 do45 do67 in2 P S0 S1 OV0 dP0 P OV1 dP1 out01 QK0 P QK1 dwo01 dx01 dwq01 in3 P
S2 S3 OV2 dP2 P OV3 dP3 out23 P QK2 QK3 in4 P S4 dwo23 dwq23 P OV4 dP4 S5 dx23 P QK4 P OV5 dP5 S6 out45 P QK5 P R
OV6 dP6 S7 dx45 P R QK6 R OV7 dP7 out67 R QK7 R dwo4567 dx67 dwq4567 R
"""
PLAN = """
.rrr.r
.r..rr.rr.r.rr..rrr.rr..rr.rr .r..rr.rr.r.rr..rrr.rr..rr.rr .r..rr.rr.r.rr..rr..rr..rr.rr
.r..rr.rr.r.rr..rrr.rr..rr.rr .RE...w..w.w...w...w..ww..w.. w..w..w..w.w...w...w..w...w..
w.....w..w.....w...w..w...w.. w..w..w....w...w...w..w...w.. w..w..w..w.w...w...w...W.....
..E.r..r..r.rr..rrr.rr..rr.rr .r..rr.rr.r.rr..rrr.rr..rr.rr .r..rr.rr.r.rr..rr..rr..rr.rr
.r..rr.rr.r.rr..rrr.rr..rr.rr .r..rr.rr.r.rr..rr..rr..rr.rr .RE...w..w.w...w...w..ww..w..
w..w..w....w...w...w..w...w.. w..w..w....w...w...w..w...... w..w..w..w.w...w...w..w...w..
w..w..w..w.....w...w..w...W.. ..E....r..r.rr..rrr.rr..rr.rr .r..rr.rr.r.rr..rrr.rr..rr.rr
.r..rr.rr.r.rr..rr..rr..rr.rr .r..rr.rr.r.rr..rrr.rr..rr.rr .r..rr.rr.r.rr..rrr.rr..rr.rr
.r..rr.rr.r.R.E....w..ww..w.. w..w..w..w.w...w...w..ww..w.. ......w..w.....w...w..w...w..
w..w..w..w.w...w...w..ww..... w..w..w....w...w...w...w..... w..w..w....w...w...w..w......
w.....w........w...w...w.....
"""
PREFETCH = (75, 20, 18, 24, 12, 16, 20, 12, 10, 16, 10, 14, 6, 12, 3, 0)


def _parse(order):
    ops = []
    for op in order.split():
        kind = op.rstrip("0123456789")
        ops.append((kind, [int(c) for c in op[len(kind):]] or list(range(G))))
    return ops


def _site_table():
    table, issued, held, used, made = [], {"R": FIRST * RQ, "W": 0}, None, {}, {}
    for n, marks in enumerate(PLAN.split()):
        needed = {"R": (2 * n + 2) * RQ, "W": (2 * n + 2 - NW) * WQ}
        assert all(issued[kind] >= needed[kind] for kind in "RW") and (held is None or held[1] >= needed[held[0]])
        row = []
        for kind, js in _parse(ORDER if n else FIRST_ORDER):
            m = 2 * n + js[0] // GB
            if kind in ("S", "OV", "dP", "QK"):
                used[m] = used.get(m, 0) + 1
                made[kind, m] = made.get((kind, m), 0) + 1
                assert made[kind, m] == js[0] % GB + 1
            elif kind in ("R", "W", "E"):
                mark = marks[len(row)]
                if mark == ".":
                    row.append(-1)
                elif kind == "E":
                    row.append(2 * held[1] + (held[0] == "W"))
                    held = None
                else:
                    t = issued[kind]
                    assert held is None and mark.upper() == kind
                    if kind == "R":
                        assert t // RQ < NR or used.get(t // RQ - NR) == 4 * GB
                    else:
                        assert made.get(("QK", t // WQ), 0) >= (t % WQ + 1) * GB // WQ
                    held = (kind, t) if mark == kind else None
                    row.append(2 * t + (mark == kind))
                    issued[kind] += 1
        assert len(row) == len(marks)
        table.append(row)
    assert len(table) == N and held is None and issued == {"R": NG * RQ, "W": NG * WQ}
    return table


SITES = _site_table()
SLOTS = [m % NR for m in range(NG)] + [m % NW for m in range(NG)] + [2 * GB * NW] * 2
WORDS = SLOTS + [entry for row in SITES[1:] for entry in row]
KV, DKV, WT, DWT, TOK, PRO, NSEM = 0, 8, 16, 32, 48, 49, 59


def _dot(a, b):
    return jnp.dot(a, b, preferred_element_type=F32)


def _dot_nt(a, b):
    return lax.dot_general(a, b, (((1,), (1,)), ((), ())), preferred_element_type=F32)


def _dot_tn(a, b):
    return lax.dot_general(a, b, (((0,), (0,)), ((), ())), preferred_element_type=F32)


def _ds(start, n, align):
    return pl.ds(start if isinstance(start, int) else pl.multiple_of(start, align), n)


def _rows(view, r, n):
    return [ref.at[pl.ds(r, n)] if ref.ndim == 2 else ref.at[:, pl.ds(r, n)] for ref in view]


def _kernel(x_h, k_h, v_h, wq_h, wo_h, g_h, out_h, dx_h, dk_h, dv_h, dwq_h, dwo_h,
            x_v, g_v, kv_v, wq_v, wo_v, dkv_v, dwq_s, st_v, out_a, dx_a, dwq_a, dwo_a,
            q_s, do_s, p_s, ds_s, o_s, dq_s, sems, tab):

    def start(copies, on=True):
        @pl.when(on)
        def _():
            for src, dst, sem, priority in copies:
                pltpu.make_async_copy(src, dst, sems.at[sem]).start(priority=priority)

    def start_many(copies, on):
        limit = jnp.where(on, len(copies), 0)
        for i in range(0, len(copies), 8):
            start(copies[i:i + 8], i < limit)

    def wait(buffers, on=True):
        @pl.when(on)
        def _():
            for ref, sem in buffers:
                pltpu.make_async_copy(ref, ref, sems.at[sem]).wait()

    def weight_views(grad, s, c, parts):
        sl, nq, no = s & (NWS - 1), D // parts, HP // parts
        return [((wq_h, dwq_h)[grad].at[_ds(c * nq, nq, 8), _ds(s * HP, HP, 128)],
                 (wq_v, dwq_s)[grad].at[_ds(sl * D + c * nq, nq, 8)]),
                ((wo_h, dwo_h)[grad].at[_ds(s * HP + c * no, no, 8)],
                 (wo_v, st_v)[grad].at[sl, _ds(c * no, no, 8)])]

    def weight_blocks(grad, sl):
        return [((wq_v, dwq_s)[grad].at[_ds(sl * D, D, D)], (WT, DWT)[grad] + sl),
                ((wo_v, st_v)[grad].at[sl, pl.ds(0, HP)], (WT, DWT)[grad] + NWS + sl)]

    def token_view(a, it):
        return (x_h, g_h)[a].at[it], (x_v, g_v)[a].at[pl.ds(it * T, T)]

    def read_views(t):
        m, n = t >> 2, HP // RQ
        sl = SLOTS[m] if isinstance(m, int) else tab[m]
        vmem = kv_v.at[pl.ds(2 * GB * sl, 2 * GB), _ds((t & 3) * n, n, n)]
        return [(hbm.at[m & 3, :, (m >> 2) * RQ + (t & 3)], vmem.at[pl.ds(a * GB, GB)])
                for a, hbm in enumerate((k_h, v_h))], KV + (sl >> 1)

    def write_views(t):
        m, h = t >> 1, t & 1
        sl = tab[NG + m]
        return [(dkv_v.at[pl.ds((2 * sl + a) * GB + 2 * h, 2)], hbm.at[m & 3, pl.ds(2 * h, 2), m >> 2])
                for a, hbm in ((1, dv_h), (0, dk_h))], DKV + (sl >> 1)

    def read(entry):
        t = (max(entry, 0) if isinstance(entry, int) else jnp.maximum(entry, 0)) >> 1
        on = entry >= 0
        views, sem = read_views(t)
        copies = [(*_rows(view, r + dr, n), sem, a) for r in range(0, HP // RQ, 32) for dr, n in ((0, 24), (24, 8))
                  for a, view in enumerate(views)]
        start(copies[:9], on)
        start(copies[9:10], on & (entry & 1 == 0))
        start(copies[10:11], on)
        start(copies[11:], on & (entry & 1 == 0))
        s = ((t >> 4) + 1) & (NS - 1)
        start([(*view, WT + a * NWS + (s & (NWS - 1)), a) for a, view in enumerate(weight_views(0, s, t & 15, 16))],
              on & (s > 0))

    def write(entry):
        t, on = jnp.maximum(entry, 0) >> 1, entry >= 0
        views, sem = write_views(t)
        copies = [(*_rows(view, r0, r1 - r0), sem, 0) for r0, r1 in zip(WRITE_CUTS, WRITE_CUTS[1:]) for view in views]
        s = ((t >> 3) - 1) & (NS - 1)
        extra = [(vmem, hbm, DWT + a * NWS + (s & (NWS - 1)), 0)
                 for a, (hbm, vmem) in enumerate(weight_views(1, s, t & 7, 8))]
        start(copies[:4], on)
        start(extra[:1], t >= 8)
        start(copies[4:-4], on)
        start(extra[1:], t >= 8)
        start(copies[-4:-1], on)
        start(copies[-1:], on & (entry & 1 == 0))

    def end_burst(entry):
        for grad, widths in enumerate(TAIL_WIDTHS):
            on = (entry >= 0) & (entry & 1 == grad)
            (_, view), sem = (read_views, write_views)[grad](jnp.where(on, entry >> 1, 0))
            nb, end = view[0].shape[:2]
            start_many([(*[ref.at[b, pl.ds(end - 8 * (len(widths) - r), 8), pl.ds(c, w)] for ref in view], sem, 1 - grad)
                        for r, w in enumerate(widths) for c in range(0, SK, w) for b in range(nb)], on)

    arrivals, pieces = [], []

    def cut(view, sem):
        *nb, end, width = view[0].shape
        unit = 8 * (GB * SK // (width * (nb[0] if nb else 1)))
        out, r = [], 0
        while r < end:
            n = min((3, 1)[len(out) % 2] * unit, end - r)
            out.append((*_rows(view, r, n), sem))
            r += n
        return out

    def fetch(views, sem0, sem1):
        one, two = cut(views[0], sem0), cut(views[1], sem1)
        pieces.extend(one[:len(one) - len(two)])
        pieces.extend(piece for pair in zip(one[-len(two):], two, strict=True) for piece in pair)

    for a in range(2):
        views = [token_view(a, 0), weight_views(0, 0, 0, 1)[a]]
        fetch(views, PRO + a, WT + a * NWS)
        arrivals.append([(views[0][1], PRO + a), (views[1][1], WT + a * NWS)])
    for i, (m, b0, nb) in enumerate([(0, 0, 2), (0, 2, 2), (1, 0, 4)]):
        for t in range(m * RQ, (m + 1) * RQ):
            views = [[ref.at[pl.ds(b0, nb)] for ref in view] for view in read_views(t)[0]]
            fetch(views, PRO + 2 + 2 * i, PRO + 3 + 2 * i)
        arrivals.append([(kv_v.at[pl.ds((2 * m + a) * GB + b0, nb)], PRO + 2 + 2 * i + a) for a in range(2)])
    fetch([token_view(0, 1), token_view(1, 1)], PRO + 8, PRO + 9)
    arrivals.append([(token_view(a, 1)[1], PRO + 8 + a) for a in range(2)])
    for t in range(2 * RQ, FIRST * RQ):
        fetch(read_views(t)[0], KV + 1, KV + 1)
    fetch(weight_views(0, 1, 0, 1), WT + 1, WT + NWS + 1)
    queue = [(*pieces[i], i % 2) for i in sorted(range(len(pieces)), key=lambda i: i - 2 * SKEW * (i % 2))]
    counts = list(PREFETCH)

    def prefetch():
        start([queue.pop(0) for _ in range(counts.pop(0))])

    prefetch()
    for acc in (out_a, dx_a):
        acc[pl.ds(T, T)] = jnp.zeros((T, D), F32)
    for i, word in enumerate(WORDS):
        tab[i] = word

    def step(n, order, read_slot, write_slot):
        first = isinstance(n, int)
        s, it = n >> 1, n & 1
        sl = s & (NWS - 1)
        wq, wo = wq_v.at[_ds(sl * D, D, D)], wo_v.at[sl]

        def blocks(ref, slot, a):
            return [ref.at[2 * GB * slot + (2 * (j // GB) + a) * GB + j % GB] for j in range(G)]

        k, v = blocks(kv_v, read_slot, 0), blocks(kv_v, read_slot, 1)
        dk, dv = blocks(dkv_v, write_slot, 0), blocks(dkv_v, write_slot, 1)
        lo = lax.broadcasted_iota(jnp.int32, (SQ, 128), 1) < 64

        def split_heads(a):
            m = a[:, 128:256]
            return jnp.concatenate([a[:, 0:128], jnp.where(lo, m, 0.0), jnp.where(lo, 0.0, m), a[:, 256:384]], 0)

        def merge_heads(r0, rm, r2):
            return jnp.concatenate([r0, jnp.where(lo, rm[0:SQ], rm[SQ:]), r2], 1)

        def scores(a, w):
            rm = _dot(a[SQ:3 * SQ], w[128:256, :])
            r0 = _dot(a[0:SQ], w[0:128, :])
            r2 = _dot(a[3 * SQ:4 * SQ], w[256:384, :])
            return jnp.concatenate([r0 + rm[0:SQ], r2 + rm[SQ:]], 0)

        def apply(p, w, a, dw):
            r0 = _dot_nt(p[0:SQ], w[0:128, :])
            while delayed:
                read(delayed.pop())
            z = jnp.zeros((SQ, 128), BF16)
            diag = jnp.concatenate([jnp.concatenate([a[0:SQ], z], 0), a[SQ:3 * SQ],
                                    jnp.concatenate([z, a[3 * SQ:]], 0)], 1)
            dw[...] = _dot_tn(diag, p[0:2 * SQ]).astype(BF16)
            rm = _dot_nt(p[0:2 * SQ], w[128:256, :])
            r2 = _dot_nt(p[SQ:2 * SQ], w[256:384, :])
            return r0, rm, r2

        def accumulate(acc, idx, stage, stage_idx, fresh, val):
            if fresh is not True:
                val = val + (acc[idx] if fresh is False else jnp.where(fresh, 0.0, acc[idx]))
            acc[idx] = val
            if not first:
                stage[stage_idx] = val.astype(BF16)

        delta, delayed, pinned, site = {}, [], False, 0
        ops = _parse(order)
        for (kind, js), (following, _) in zip(ops, ops[1:] + [(None, None)]):
            j = js[0]
            own = pl.ds(j * SQ, len(js) * SQ)
            tok = _ds(it * T + j * SQ, len(js) * SQ, SQ)
            q, do, p, ds = q_s.at[j], do_s.at[j], p_s.at[j], ds_s.at[j]
            if kind in ("R", "W", "E"):
                entry = SITES[0][site] if first else tab[len(SLOTS) + (n - 1) * len(SITES[1]) + site]
                site += 1
                if kind == "R" and following in ("OV", "QK"):
                    delayed.append(entry)
                else:
                    {"R": read, "W": write, "E": end_burst}[kind](entry)
            elif kind == "in":
                assert not any(copy[2] == sem for copy in queue for _, sem in arrivals[j])
                wait(arrivals[j])
            elif kind == "P":
                prefetch()
            elif kind == "fin":
                start_many([(st_v.at[NWS + 2 * a + it, pl.ds(r, 32)], hbm.at[it, pl.ds(r, 32)], TOK, 0)
                            for r in range(0, T, 32) for a, hbm in enumerate((out_h, dx_h))], s == NS - 1)
            elif kind == "pin":
                pinned = True
            elif kind in ("q", "do"):
                r = _dot(x_v[tok, :], wq[...]) * DH ** -0.5 if kind == "q" else _dot_nt(g_v[tok, :], wo[...])
                for i, jj in enumerate(js):
                    (q_s if kind == "q" else do_s)[jj] = split_heads(r[i * SQ:(i + 1) * SQ]).astype(BF16)
            elif kind == "S":
                t = scores(q, k[j])
                e = jnp.exp(t - jnp.max(t, axis=1, keepdims=True))
                p[...] = (e * (1.0 / jnp.sum(e, axis=1, keepdims=True))).astype(BF16)
            elif kind == "OV":
                r = apply(p, v[j], do, dv[j])
                o_s[own] = merge_heads(*r).astype(BF16)
                t = jnp.concatenate(r, 0) * do[...].astype(F32)
                t = jnp.concatenate([t[0:SQ] + t[SQ:2 * SQ], t[2 * SQ:3 * SQ] + t[3 * SQ:]], 0)
                delta[j] = jnp.sum(t, axis=1, keepdims=True)
            elif kind == "dP":
                ds[...] = (p[...].astype(F32) * (scores(do, v[j]) - delta[j])).astype(BF16)
            elif kind == "QK":
                dq_s[own] = (merge_heads(*apply(ds, k[j], q, dk[j])) * DH ** -0.5).astype(BF16)
            else:
                a = (o_s if kind in ("out", "dwo") else dq_s)[own]
                if pinned:
                    dkv_v[tab[2 * NG], 0:a.shape[0], 0:HP] = a
                    a = dkv_v[tab[2 * NG + 1], 0:a.shape[0], 0:HP]
                    pinned = False
                if kind == "out":
                    accumulate(out_a, tok, st_v, (NWS + it, own), first, _dot(a, wo[...]))
                elif kind == "dx":
                    accumulate(dx_a, tok, st_v, (NWS + 2 + it, own), first, _dot_nt(a, wq[...]))
                elif kind == "dwo":
                    accumulate(dwo_a, ..., st_v, (sl, pl.ds(0, HP)), j == 0 and it == 0, _dot_tn(a, g_v[tok, :]))
                else:
                    accumulate(dwq_a, ..., dwq_s, _ds(sl * D, D, D), j == 0 and it == 0, _dot_tn(x_v[tok, :], a))

    step(0, FIRST_ORDER, 0, 0)
    assert not queue
    wait(arrivals[-1])

    def loop(n, slots):
        rs, ws = slots
        wait([(kv_v.at[pl.ds(2 * GB * rs, 2 * G)], KV + (rs >> 1))])
        wait([(dkv_v.at[pl.ds(2 * GB * ws, 2 * G)], DKV + (ws >> 1))], 2 * n >= NW)
        wait(weight_blocks(0, (n >> 1) & (NWS - 1)), (n & 1) == 0)
        wait(weight_blocks(1, (n >> 1) & (NWS - 1)), ((n & 1) == 0) & (n >= 2 * NWS))
        step(n, ORDER, rs, ws)
        return jnp.where(rs + 2 == NR, 0, rs + 2), jnp.where(ws + 2 == NW, 0, ws + 2)

    lax.fori_loop(1, N, loop, (jnp.int32(2), jnp.int32(2)))
    start([(vmem, hbm, DWT + a * NWS + NWS - 1, 0)
           for c in range(8) for a, (hbm, vmem) in enumerate(weight_views(1, NS - 1, c, 8))])
    wait([(dkv_v.at[pl.ds(2 * GB * sl, 2 * G)], DKV + sl // 2) for sl in range(0, NW, 2)])
    wait([(st_v.at[pl.ds(NWS, 4)], TOK)] + [block for sl in range(NWS) for block in weight_blocks(1, sl)])


@jax.jit
def pallas_standalone__gqa_block_cached__near_ridge_kernel(
    x: jax.Array,
    k_cache: jax.Array,
    v_cache: jax.Array,
    wq: jax.Array,
    wo: jax.Array,
    grad_out: jax.Array,
):
    assert x.shape == (B, SQ, D) and k_cache.shape == v_cache.shape == (B, H, SK, DH)

    def keys_last(a):
        return jnp.swapaxes(a, 2, 3).reshape(B // GB, GB, NS * RQ, HP // RQ, SK)

    def keys_first(a):
        return jnp.swapaxes(a.reshape(B, H, DH, SK), 2, 3)

    hbm = pl.BlockSpec(memory_space=pl.ANY)
    shapes = [(2, T, D)] * 2 + [(B // GB, GB, NS, HP, SK)] * 2 + [wq.shape, wo.shape]
    out, dx, dk, dv, dwq, dwo = pl.pallas_call(
        _kernel,
        in_specs=[hbm] * 6,
        out_specs=[hbm] * 6,
        out_shape=[jax.ShapeDtypeStruct(shape, BF16) for shape in shapes],
        scratch_shapes=[
            pltpu.VMEM((B * SQ, D), BF16), pltpu.VMEM((B * SQ, D), BF16),
            pltpu.VMEM((2 * GB * NR, HP, SK), BF16),
            pltpu.VMEM((NWS * D, HP), BF16), pltpu.VMEM((NWS, HP, D), BF16),
            pltpu.VMEM((2 * GB * NW + 1, HP, SK), BF16),
            pltpu.VMEM((NWS * D, HP), BF16), pltpu.VMEM((NWS + 4, T, D), BF16),
            pltpu.VMEM((B * SQ, D), F32), pltpu.VMEM((B * SQ, D), F32),
            pltpu.VMEM((D, HP), F32), pltpu.VMEM((HP, D), F32),
            pltpu.VMEM((G, 4 * SQ, 128), BF16), pltpu.VMEM((G, 4 * SQ, 128), BF16),
            pltpu.VMEM((G, 2 * SQ, SK), BF16), pltpu.VMEM((G, 2 * SQ, SK), BF16),
            pltpu.VMEM((T, HP), BF16), pltpu.VMEM((T, HP), BF16),
            pltpu.SemaphoreType.DMA((NSEM,)), pltpu.SMEM((len(WORDS),), jnp.int32),
        ],
        compiler_params=pltpu.CompilerParams(
            vmem_limit_bytes=127 * 2 ** 20, disable_bounds_checks=True, disable_semaphore_checks=True),
    )(x.reshape(2, T, D), keys_last(k_cache), keys_last(v_cache), wq, wo, grad_out.reshape(2, T, D))
    return out.reshape(B, SQ, D), dx.reshape(B, SQ, D), keys_first(dk), keys_first(dv), dwq, dwo
```
